```python
import os as _os
_os.environ.setdefault("JAX_PLATFORMS", "cpu")
import jax
import jax.numpy as jnp

def _softmax(x, axis=-1):
    return jax.nn.softmax(x, axis=axis)
def _gelu(x):
    return jax.nn.gelu(x, approximate=True)
def _silu(x):
    return jax.nn.silu(x)
def _sigmoid(x):
    return jax.nn.sigmoid(x)
def _layernorm(x, axis=-1, eps=1e-5):
    m = jnp.mean(x, axis=axis, keepdims=True)
    v = jnp.var(x, axis=axis, keepdims=True)
    return (x - m) / jnp.sqrt(v + eps)
def _scatter_add(tgt, idx, src, axis=0):
    return tgt.at[idx].add(src)
def _segment_sum(src, seg, n):
    return jax.ops.segment_sum(src, seg, n)
class _Rng:
    def __init__(self, key):
        self._k = key
    def _next(self):
        self._k, sub = jax.random.split(self._k)
        return sub
    def normal(self, shape):
        return jax.random.normal(self._next(), shape, dtype=jnp.bfloat16)
    def randint(self, lo, hi, shape):
        return jax.random.randint(self._next(), shape, lo, hi, dtype=jnp.int32)
    def uniform(self, shape, lo=0.0, hi=1.0):
        return jax.random.uniform(self._next(), shape, jnp.bfloat16, lo, hi)
    def permutation(self, n):
        return jax.random.permutation(self._next(), n)


kernel_name = 'concat_heads__gqa_block_cached__gqa_block_cached__near_ridge'

def setup_inputs():
    _rng = _Rng(jax.random.key(int.from_bytes(__import__("os").urandom(4), "little")))
    _w = (lambda a: (lambda t: t.astype(jnp.bfloat16) if jnp.issubdtype(t.dtype, jnp.floating) else t)(jnp.asarray(a)))
    def _A_setup():
        B, Sq, D = 8, 128, 576
        Hq, Hkv, Sk, Dh = 32, 16, 512, 128
        assert Hq % Hkv == 0, (Hq, Hkv)
        return {
            "x": _w((lambda *s: _rng.normal(s) * 0.8)(B, Sq, D)),
            "k_cache": _w((lambda *s: _rng.normal(s) * 0.8)(B, Hkv, Sk, Dh)),
            "v_cache": _w((lambda *s: _rng.normal(s) * 0.05)(B, Hkv, Sk, Dh)),
            "wq": _w((lambda *s: _rng.normal(s) * 0.8)(D, Hq * Dh) * (D ** -0.5)),
            "wo": _w((lambda *s: _rng.normal(s) * 0.05)(Hq * Dh, D) * ((Hq * Dh) ** -0.5)),
        }
    _A_in = _A_setup()

    def _B_setup():
        B, Sq, D = 8, 128, 576
        Hq, Hkv, Sk, Dh = 32, 16, 512, 128
        assert Hq % Hkv == 0, (Hq, Hkv)
        return {
            "x": _w((lambda *s: _rng.normal(s) * 0.8)(B, Sq, D)),
            "k_cache": _w((lambda *s: _rng.normal(s) * 0.8)(B, Hkv, Sk, Dh)),
            "v_cache": _w((lambda *s: _rng.normal(s) * 0.05)(B, Hkv, Sk, Dh)),
            "wq": _w((lambda *s: _rng.normal(s) * 0.8)(D, Hq * Dh) * (D ** -0.5)),
            "wo": _w((lambda *s: _rng.normal(s) * 0.05)(Hq * Dh, D) * ((Hq * Dh) ** -0.5)),
        }
    _B_in = _B_setup()

    return {
        "A_x": _A_in["x"],
        "A_k_cache": _A_in["k_cache"],
        "A_v_cache": _A_in["v_cache"],
        "A_wq": _A_in["wq"],
        "A_wo": _A_in["wo"],
        "B_x": _B_in["x"],
        "B_k_cache": _B_in["k_cache"],
        "B_v_cache": _B_in["v_cache"],
        "B_wq": _B_in["wq"],
        "B_wo": _B_in["wo"],
    }

def reference(A_x, A_k_cache, A_v_cache, A_wq, A_wo, B_x, B_k_cache, B_v_cache, B_wq, B_wo):
    def _A_ref(x, k_cache, v_cache, wq, wo):
        B, Sq, D = x.shape
        Hq, Dh = 32, 128
        Hkv = k_cache.shape[1]
        rep = Hq // Hkv
        q = (lambda x, *d: x.transpose(*d))((x @ wq).reshape(B, Sq, Hq, Dh), 0, 2, 1, 3)
        k = jnp.repeat(k_cache, rep, axis=1)
        v = jnp.repeat(v_cache, rep, axis=1)
        scores = jnp.einsum("bhqd,bhkd->bhqk", q, k) * (Dh ** -0.5)
        p = _softmax(scores, axis=-1)
        o = jnp.einsum("bhqk,bhkd->bhqd", p, v)
        return (lambda x, *d: x.transpose(*d))(o, 0, 2, 1, 3).reshape(B, Sq, Hq * Dh) @ wo

    def _B_ref(x, k_cache, v_cache, wq, wo):
        B, Sq, D = x.shape
        Hq, Dh = 32, 128
        Hkv = k_cache.shape[1]
        rep = Hq // Hkv
        q = (lambda x, *d: x.transpose(*d))((x @ wq).reshape(B, Sq, Hq, Dh), 0, 2, 1, 3)
        k = jnp.repeat(k_cache, rep, axis=1)
        v = jnp.repeat(v_cache, rep, axis=1)
        scores = jnp.einsum("bhqd,bhkd->bhqk", q, k) * (Dh ** -0.5)
        p = _softmax(scores, axis=-1)
        o = jnp.einsum("bhqk,bhkd->bhqd", p, v)
        return (lambda x, *d: x.transpose(*d))(o, 0, 2, 1, 3).reshape(B, Sq, Hq * Dh) @ wo

    a = _A_ref(A_x, A_k_cache, A_v_cache, A_wq, A_wo)
    b = _B_ref(B_x, B_k_cache, B_v_cache, B_wq, B_wo)
    return jnp.concatenate([a, b], axis=-1)
```

```python
import math

import jax
import jax.numpy as jnp
import numpy as np
from jax.experimental import pallas as pl
from jax.experimental.pallas import tpu as pltpu

B, SQ, D = 8, 128, 576
HQ, HKV, SK, DH = 32, 16, 512, 128
R = B * SQ
NSTEP = 2 * HKV
NB = 4
U = 2
P = 3
SCALE = float(DH ** -0.5 * math.log2(math.e))
BF = jnp.bfloat16
F32 = jnp.float32
NT = (((1,), (1,)), ((), ()))
KINDS = ("wq", "k", "v", "wo")


def _kernel(xA, kA, vA, wqA, woA, xB, kB, vB, wqB, woB, out_hbm,
            xT_s, x_s, wq_s, wo_s, k_s, v_s, q_s, o_s, acc, out_s,
            sem_x, sem_wq, sem_wo, sem_k, sem_v, sem_out):
    halves = ((xB, kB, vB, wqB, woB), (xA, kA, vA, wqA, woA))

    def copy(kind, h, hk, slot):
        x, k, v, wq, wo = halves[h]
        if kind == "wq":
            return pltpu.make_async_copy(wq.at[:, pl.ds(hk * 256, 256)], wq_s.at[slot], sem_wq.at[slot])
        if kind == "wo":
            return pltpu.make_async_copy(wo.at[:, pl.ds(hk * 256, 256)], wo_s.at[slot], sem_wo.at[slot])
        if kind == "k":
            return pltpu.make_async_copy(k.at[:, hk], k_s.at[slot], sem_k.at[slot])
        return pltpu.make_async_copy(v.at[:, hk], v_s.at[slot], sem_v.at[slot])

    def start(kind, t):
        if isinstance(t, int):
            if t < NSTEP:
                copy(kind, t // HKV, t % HKV, t % NB).start()
            return
        hk = t & (HKV - 1)
        slot = t & (NB - 1)

        @pl.when(t < HKV)
        def _():
            copy(kind, 0, hk, slot).start()

        @pl.when(jnp.logical_and(t >= HKV, t < NSTEP))
        def _():
            copy(kind, 1, hk, slot).start()

    def wait(kind, t):
        slot = t % NB if isinstance(t, int) else t & (NB - 1)
        copy(kind, 0, 0, slot).wait()

    def half_slot(t):
        if isinstance(t, int):
            return t // HKV, t % NB
        return t >> 4, t & (NB - 1)

    def x_part(h, lo, hi, sem):
        return pltpu.make_async_copy(halves[h][0].at[pl.ds(lo, hi - lo)], xT_s.at[h, pl.ds(lo, hi - lo)],
                                     sem_x.at[sem])

    def kv_part(kind, lo, hi, sem):
        src = halves[0][1 if kind == "k" else 2]
        dst = k_s if kind == "k" else v_s
        return pltpu.make_async_copy(src.at[pl.ds(lo, hi - lo), 0], dst.at[0, pl.ds(lo, hi - lo)], sem_x.at[sem])

    def xpose_x(h, lo, hi):
        for b in range(lo, hi):
            x_s[h, pl.ds(b * SQ, SQ), :] = xT_s[h, b].T

    def qproj_chunk(t, c):
        half, slot = half_slot(t)
        rows = pl.ds(c * (R // 2), R // 2)
        q = jnp.dot(x_s[half, rows, :], wq_s[slot], preferred_element_type=F32) * SCALE
        q = q.astype(BF)
        q_s[0, rows, :] = q[:, :DH]
        q_s[1, rows, :] = q[:, DH:]

    def qproj(t):
        qproj_chunk(t, 0)
        qproj_chunk(t, 1)

    def attn_scores(t, b):
        _, slot = half_slot(t)
        rows = pl.ds(b * SQ, SQ)
        q = jnp.concatenate([q_s[0, rows, :], q_s[1, rows, :]], axis=0)
        s = jax.lax.dot_general(q, k_s[slot, b], NT, preferred_element_type=F32)
        m = jnp.max(s, axis=1, keepdims=True)
        p = jnp.exp2(s - m)
        l = jnp.sum(p, axis=1, keepdims=True)
        r = pltpu.reciprocal(l, approx=True)
        r = r * (2.0 - l * r)
        return p.astype(BF), r

    def attn_values(t, b, pr):
        _, slot = half_slot(t)
        rows = pl.ds(b * SQ, SQ)
        p, r = pr
        o = jnp.dot(p, v_s[slot, b], preferred_element_type=F32)
        o = (o * r).astype(BF)
        o_s[0, rows, :] = o[:SQ]
        o_s[1, rows, :] = o[SQ:]

    def attn(t, lo=0, hi=B):
        pr = {}
        for b in range(lo, hi + 1):
            if b < hi:
                pr[b] = attn_scores(t, b)
            if b > lo:
                attn_values(t, b - 1, pr.pop(b - 1))

    def oproj(t):
        half, slot = half_slot(t)
        o = jnp.concatenate([o_s[0], o_s[1]], axis=1)
        acc[1 - half] += jax.lax.dot_general(wo_s[slot], o, NT, preferred_element_type=F32)

    xb0, xb1, xa = x_part(0, 0, 4, 0), x_part(0, 4, 8, 1), x_part(1, 0, 8, 2)
    k0a, v0a = kv_part("k", 0, 4, 3), kv_part("v", 0, 4, 4)
    k0b, v0b = kv_part("k", 4, 8, 5), kv_part("v", 4, 8, 6)
    xb0.start()
    start("wq", 0)
    xb1.start()
    acc[...] = jnp.zeros(acc.shape, F32)
    xb0.wait()
    wait("wq", 0)
    k0a.start()
    v0a.start()
    xpose_x(0, 0, 4)
    qproj_chunk(0, 0)
    xb1.wait()
    k0b.start()
    v0b.start()
    xpose_x(0, 4, 8)
    qproj_chunk(0, 1)
    k0a.wait()
    v0a.wait()
    start("wo", 0)
    start("wq", 1)
    attn(0, 0, 4)
    k0b.wait()
    v0b.wait()
    wait("wo", 0)
    start("k", 1)
    start("v", 1)
    attn(0, 4, 8)
    start("wo", 1)
    start("wq", 2)
    oproj(0)
    wait("wq", 1)
    start("k", 2)
    xa.start()
    qproj(1)
    wait("k", 1)
    wait("v", 1)
    wait("wo", 1)
    start("v", 2)
    start("wo", 2)
    attn(1, 0, 4)
    start("wq", 3)
    start("k", 3)
    attn(1, 4, 8)
    oproj(1)
    for kind in KINDS:
        wait(kind, 2)
    xa.wait()
    start("v", 3)
    start("wo", 3)
    xpose_x(1, 0, 8)
    qproj(2)
    for kind in KINDS:
        start(kind, 4)
    attn(2)
    oproj(2)

    def loop_body(i, carry):
        t0 = P + i * U
        for u in range(U):
            for kind in KINDS:
                wait(kind, t0 + u)
        for u in range(U):
            for kind in KINDS:
                start(kind, t0 + u + U)
        for u in range(U):
            qproj(t0 + u)
            attn(t0 + u)
            oproj(t0 + u)
        return carry

    jax.lax.fori_loop(0, (NSTEP - 1 - P) // U, loop_body, None)

    t = NSTEP - 1
    slot = t % NB
    wait("wq", t)
    for b in range(B):
        rows = pl.ds(b * SQ, SQ)
        out_s[rows, 640:1152] = acc[1, 64:576, rows].astype(BF).T
    copy_b = pltpu.make_async_copy(out_s.at[:, pl.ds(640, 512)], out_hbm.at[:, pl.ds(640, 512)], sem_out.at[0])
    copy_b.start()
    qproj(t)
    wait("k", t)
    wait("v", t)
    wait("wo", t)

    def finish(b):
        rows = pl.ds(b * SQ, SQ)
        o = jnp.concatenate([o_s[0, rows, :], o_s[1, rows, :]], axis=1)
        parts = []
        for r in range(2):
            rr = pl.ds(r * (D // 2), D // 2)
            parts.append(acc[0, rr, rows]
                         + jax.lax.dot_general(wo_s[slot, rr, :], o, NT, preferred_element_type=F32))
        out_t = jnp.concatenate(parts + [acc[1, 0:64, rows]], axis=0).astype(BF)
        out_s[rows, 0:640] = out_t.T
        pltpu.make_async_copy(out_s.at[rows, pl.ds(0, 640)], out_hbm.at[rows, pl.ds(0, 640)], sem_out.at[1]).start()

    pr = {}
    for b in range(B + 3):
        if b < B:
            pr[b] = attn_scores(t, b)
        if 1 <= b <= B:
            attn_values(t, b - 1, pr.pop(b - 1))
        if b >= 3:
            finish(b - 3)
    copy_b.wait()
    pltpu.make_async_copy(out_s.at[:, pl.ds(0, 640)], out_hbm.at[:, pl.ds(0, 640)], sem_out.at[1]).wait()


@jax.jit
def pallas_concat_heads__gqa_block_cached__gqa_block_cached__near_ridge_kernel(
    A_x: jax.Array,
    A_k_cache: jax.Array,
    A_v_cache: jax.Array,
    A_wq: jax.Array,
    A_wo: jax.Array,
    B_x: jax.Array,
    B_k_cache: jax.Array,
    B_v_cache: jax.Array,
    B_wq: jax.Array,
    B_wo: jax.Array,
):
    hbm = pl.BlockSpec(memory_space=pltpu.HBM)
    out = pl.pallas_call(
        _kernel,
        out_shape=jax.ShapeDtypeStruct((R, 2 * D), BF),
        in_specs=[hbm] * 10,
        out_specs=hbm,
        scratch_shapes=[
            pltpu.VMEM((2, B, D, SQ), BF),
            pltpu.VMEM((2, R, D), BF),
            pltpu.VMEM((NB, D, 256), BF),
            pltpu.VMEM((NB, D, 256), BF),
            pltpu.VMEM((NB, B, SK, DH), BF),
            pltpu.VMEM((NB, B, SK, DH), BF),
            pltpu.VMEM((2, R, DH), BF),
            pltpu.VMEM((2, R, DH), BF),
            pltpu.VMEM((2, D, R), F32),
            pltpu.VMEM((R, 2 * D), BF),
            pltpu.SemaphoreType.DMA((7,)),
            pltpu.SemaphoreType.DMA((NB,)),
            pltpu.SemaphoreType.DMA((NB,)),
            pltpu.SemaphoreType.DMA((NB,)),
            pltpu.SemaphoreType.DMA((NB,)),
            pltpu.SemaphoreType.DMA((2,)),
        ],
        compiler_params=pltpu.CompilerParams(vmem_limit_bytes=64 * 1024 * 1024, disable_bounds_checks=True),
    )(jnp.transpose(A_x, (0, 2, 1)), A_k_cache, A_v_cache, A_wq, A_wo.T,
      jnp.transpose(B_x, (0, 2, 1)), B_k_cache, B_v_cache, B_wq, B_wo.T)
    return out.reshape(B, SQ, 2 * D)
```

```python
import math

import jax
import jax.numpy as jnp
from jax.experimental import pallas as pl
from jax.experimental.pallas import tpu as pltpu

B, SQ, D = 8, 128, 576
HQ, HKV, SK, DH = 32, 16, 512, 128
R = B * SQ
NSTEP = 2 * HKV
NB = 4
U = 2
P = 3
SCALE = float(DH ** -0.5 * math.log2(math.e))
BF = jnp.bfloat16
F32 = jnp.float32
U32 = jnp.uint32
NT = (((1,), (1,)), ((), ()))
KINDS = ("wq", "k", "v", "wo")


def _kernel(xA, kA, vA, wqA, woA, xB, kB, vB, wqB, woB, out_hbm,
            xT_s, x_s, wq_s, wo_s, k_s, v_s, q_s, o_s, acc, out_s,
            sem_x, sem_wq, sem_wo, sem_k, sem_v, sem_out):
    halves = ((xB, kB, vB, wqB, woB), (xA, kA, vA, wqA, woA))

    def copy(kind, h, hk, slot):
        x, k, v, wq, wo = halves[h]
        if kind == "wq":
            return pltpu.make_async_copy(wq.at[:, pl.ds(hk * 256, 256)], wq_s.at[slot], sem_wq.at[slot])
        if kind == "wo":
            return pltpu.make_async_copy(wo.at[:, pl.ds(hk * 256, 256)], wo_s.at[slot], sem_wo.at[slot])
        if kind == "k":
            return pltpu.make_async_copy(k.at[:, hk], k_s.at[slot], sem_k.at[slot])
        return pltpu.make_async_copy(v.at[:, hk], v_s.at[slot], sem_v.at[slot])

    def start(kind, t):
        if isinstance(t, int):
            if t < NSTEP:
                copy(kind, t // HKV, t % HKV, t % NB).start()
            return
        hk = t & (HKV - 1)
        slot = t & (NB - 1)

        @pl.when(t < HKV)
        def _():
            copy(kind, 0, hk, slot).start()

        @pl.when(jnp.logical_and(t >= HKV, t < NSTEP))
        def _():
            copy(kind, 1, hk, slot).start()

    def wait(kind, t):
        slot = t % NB if isinstance(t, int) else t & (NB - 1)
        copy(kind, 0, 0, slot).wait()

    def half_slot(t):
        if isinstance(t, int):
            return t // HKV, t % NB
        return t >> 4, t & (NB - 1)

    def x_part(h, lo, hi, sem):
        return pltpu.make_async_copy(halves[h][0].at[pl.ds(lo, hi - lo)], xT_s.at[h, pl.ds(lo, hi - lo)],
                                     sem_x.at[sem])

    def kv_part(kind, lo, hi, sem):
        src = halves[0][1 if kind == "k" else 2]
        dst = k_s if kind == "k" else v_s
        return pltpu.make_async_copy(src.at[pl.ds(lo, hi - lo), 0], dst.at[0, pl.ds(lo, hi - lo)], sem_x.at[sem])

    def xpose_x(h, lo, hi):
        for b in range(lo, hi):
            x_s[h, pl.ds(b * SQ, SQ), :] = xT_s[h, b].T

    def st32(ref, h, r0, val):
        ref[h, pl.ds(r0 // 2, val.shape[0] // 2), :] = pltpu.bitcast(val, U32)

    def ld32(ref, h, r0, n):
        return pltpu.bitcast(ref[h, pl.ds(r0 // 2, n // 2), :], BF)

    def qproj_chunk(t, c, nchunk):
        half, slot = half_slot(t)
        n = R // nchunk
        q = jnp.dot(x_s[half, pl.ds(c * n, n), :], wq_s[slot], preferred_element_type=F32) * SCALE
        q = q.astype(BF)
        st32(q_s, 0, c * n, q[:, :DH])
        st32(q_s, 1, c * n, q[:, DH:])

    def qproj(t):
        qproj_chunk(t, 0, 2)
        qproj_chunk(t, 1, 2)

    def attn_scores(t, b):
        _, slot = half_slot(t)
        q = jnp.concatenate([ld32(q_s, 0, b * SQ, SQ), ld32(q_s, 1, b * SQ, SQ)], axis=0)
        s = jax.lax.dot_general(q, k_s[slot, b], NT, preferred_element_type=F32)
        m = jnp.max(s, axis=1, keepdims=True)
        p = jnp.exp2(s - m)
        l = jnp.sum(p, axis=1, keepdims=True)
        r = pltpu.reciprocal(l, approx=True)
        r = r * (2.0 - l * r)
        return p.astype(BF), r

    def attn_values(t, b, pr):
        _, slot = half_slot(t)
        p, r = pr
        o = jnp.dot(p, v_s[slot, b], preferred_element_type=F32)
        o = (o * r).astype(BF)
        st32(o_s, 0, b * SQ, o[:SQ])
        st32(o_s, 1, b * SQ, o[SQ:])

    def attn(t, lo=0, hi=B):
        pr = {}
        for b in range(lo, hi + 1):
            if b < hi:
                pr[b] = attn_scores(t, b)
            if b > lo:
                attn_values(t, b - 1, pr.pop(b - 1))

    def oproj(t):
        half, slot = half_slot(t)
        o = jnp.concatenate([ld32(o_s, 0, 0, R), ld32(o_s, 1, 0, R)], axis=1)
        acc[1 - half] += jax.lax.dot_general(wo_s[slot], o, NT, preferred_element_type=F32)

    xb0, xb1, xa = x_part(0, 0, 4, 0), x_part(0, 4, 8, 1), x_part(1, 0, 8, 2)
    k0a, v0a = kv_part("k", 0, 4, 3), kv_part("v", 0, 4, 4)
    k0b, v0b = kv_part("k", 4, 8, 5), kv_part("v", 4, 8, 6)
    xb0.start()
    start("wq", 0)
    xb1.start()
    acc[...] = jnp.zeros(acc.shape, F32)
    xb0.wait()
    wait("wq", 0)
    k0a.start()
    v0a.start()
    xpose_x(0, 0, 4)
    for b in range(0, 4):
        qproj_chunk(0, b, B)
    xb1.wait()
    k0b.start()
    v0b.start()
    xpose_x(0, 4, 8)
    for b in range(4, 8):
        qproj_chunk(0, b, B)
    k0a.wait()
    v0a.wait()
    start("wo", 0)
    start("wq", 1)
    attn(0, 0, 4)
    k0b.wait()
    v0b.wait()
    wait("wo", 0)
    start("k", 1)
    start("v", 1)
    attn(0, 4, 8)
    start("wo", 1)
    start("wq", 2)
    oproj(0)
    wait("wq", 1)
    start("k", 2)
    xa.start()
    qproj(1)
    wait("k", 1)
    wait("v", 1)
    wait("wo", 1)
    start("v", 2)
    start("wo", 2)
    attn(1, 0, 4)
    start("wq", 3)
    start("k", 3)
    attn(1, 4, 8)
    oproj(1)
    for kind in KINDS:
        wait(kind, 2)
    xa.wait()
    start("v", 3)
    start("wo", 3)
    xpose_x(1, 0, 8)
    qproj(2)
    for kind in KINDS:
        start(kind, 4)
    attn(2)
    oproj(2)

    def loop_body(i, carry):
        t0 = P + i * U
        for u in range(U):
            for kind in KINDS:
                wait(kind, t0 + u)
        for u in range(U):
            for kind in KINDS:
                start(kind, t0 + u + U)
        for u in range(U):
            qproj(t0 + u)
            attn(t0 + u)
            oproj(t0 + u)
        return carry

    jax.lax.fori_loop(0, (NSTEP - 1 - P) // U, loop_body, None)

    t = NSTEP - 1
    slot = t % NB
    wait("wq", t)
    for b in range(B):
        rows = pl.ds(b * SQ, SQ)
        out_s[rows, 640:1152] = acc[1, 64:576, rows].astype(BF).T
    copy_b = pltpu.make_async_copy(out_s.at[:, pl.ds(640, 512)], out_hbm.at[:, pl.ds(640, 512)], sem_out.at[0])
    copy_b.start()
    qproj(t)
    wait("k", t)
    wait("v", t)
    wait("wo", t)

    def finish(b):
        rows = pl.ds(b * SQ, SQ)
        o = jnp.concatenate([ld32(o_s, 0, b * SQ, SQ), ld32(o_s, 1, b * SQ, SQ)], axis=1)
        parts = []
        for r in range(2):
            rr = pl.ds(r * (D // 2), D // 2)
            parts.append(acc[0, rr, rows]
                         + jax.lax.dot_general(wo_s[slot, rr, :], o, NT, preferred_element_type=F32))
        out_t = jnp.concatenate(parts + [acc[1, 0:64, rows]], axis=0).astype(BF)
        out_s[rows, 0:640] = out_t.T
        pltpu.make_async_copy(out_s.at[rows, pl.ds(0, 640)], out_hbm.at[rows, pl.ds(0, 640)], sem_out.at[1]).start()

    pr = {}
    for b in range(B + 3):
        if b < B:
            pr[b] = attn_scores(t, b)
        if 1 <= b <= B:
            attn_values(t, b - 1, pr.pop(b - 1))
        if b >= 3:
            finish(b - 3)
    copy_b.wait()
    pltpu.make_async_copy(out_s.at[:, pl.ds(0, 640)], out_hbm.at[:, pl.ds(0, 640)], sem_out.at[1]).wait()


@jax.jit
def pallas_concat_heads__gqa_block_cached__gqa_block_cached__near_ridge_kernel(
    A_x: jax.Array,
    A_k_cache: jax.Array,
    A_v_cache: jax.Array,
    A_wq: jax.Array,
    A_wo: jax.Array,
    B_x: jax.Array,
    B_k_cache: jax.Array,
    B_v_cache: jax.Array,
    B_wq: jax.Array,
    B_wo: jax.Array,
):
    hbm = pl.BlockSpec(memory_space=pltpu.HBM)
    out = pl.pallas_call(
        _kernel,
        out_shape=jax.ShapeDtypeStruct((R, 2 * D), BF),
        in_specs=[hbm] * 10,
        out_specs=hbm,
        scratch_shapes=[
            pltpu.VMEM((2, B, D, SQ), BF),
            pltpu.VMEM((2, R, D), BF),
            pltpu.VMEM((NB, D, 256), BF),
            pltpu.VMEM((NB, D, 256), BF),
            pltpu.VMEM((NB, B, SK, DH), BF),
            pltpu.VMEM((NB, B, SK, DH), BF),
            pltpu.VMEM((2, R // 2, DH), U32),
            pltpu.VMEM((2, R // 2, DH), U32),
            pltpu.VMEM((2, D, R), F32),
            pltpu.VMEM((R, 2 * D), BF),
            pltpu.SemaphoreType.DMA((7,)),
            pltpu.SemaphoreType.DMA((NB,)),
            pltpu.SemaphoreType.DMA((NB,)),
            pltpu.SemaphoreType.DMA((NB,)),
            pltpu.SemaphoreType.DMA((NB,)),
            pltpu.SemaphoreType.DMA((2,)),
        ],
        compiler_params=pltpu.CompilerParams(vmem_limit_bytes=64 * 1024 * 1024, disable_bounds_checks=True),
    )(jnp.transpose(A_x, (0, 2, 1)), A_k_cache, A_v_cache, A_wq, A_wo.T,
      jnp.transpose(B_x, (0, 2, 1)), B_k_cache, B_v_cache, B_wq, B_wo.T)
    return out.reshape(B, SQ, 2 * D)
```

```python
import math

import jax
import jax.numpy as jnp
from jax.experimental import pallas as pl
from jax.experimental.pallas import tpu as pltpu

B, SQ, D = 8, 128, 576
HQ, HKV, SK, DH = 32, 16, 512, 128
R = B * SQ
NSTEP = 2 * HKV
NB = 4
U = 2
P = 3
SCALE = float(DH ** -0.5 * math.log2(math.e))
BF = jnp.bfloat16
F32 = jnp.float32
U32 = jnp.uint32
NT = (((1,), (1,)), ((), ()))
KINDS = ("wq", "k", "v", "wo")


def _kernel(xA, kA, vA, wqA, woA, xB, kB, vB, wqB, woB, out_hbm,
            xT_s, x_s, wq_s, wo_s, k_s, v_s, q_s, o_s, acc, out_s,
            sem_x, sem_wq, sem_wo, sem_k, sem_v, sem_out):
    halves = ((xB, kB, vB, wqB, woB), (xA, kA, vA, wqA, woA))

    def copy(kind, h, hk, slot):
        x, k, v, wq, wo = halves[h]
        if kind == "wq":
            return pltpu.make_async_copy(wq.at[:, pl.ds(hk * 256, 256)], wq_s.at[slot], sem_wq.at[slot])
        if kind == "wo":
            return pltpu.make_async_copy(wo.at[:, pl.ds(hk * 256, 256)], wo_s.at[slot], sem_wo.at[slot])
        if kind == "k":
            return pltpu.make_async_copy(k.at[:, hk], k_s.at[slot], sem_k.at[slot])
        return pltpu.make_async_copy(v.at[:, hk], v_s.at[slot], sem_v.at[slot])

    def start(kind, t):
        if isinstance(t, int):
            if t < NSTEP:
                copy(kind, t // HKV, t % HKV, t % NB).start()
            return
        hk = t & (HKV - 1)
        slot = t & (NB - 1)

        @pl.when(t < HKV)
        def _():
            copy(kind, 0, hk, slot).start()

        @pl.when(jnp.logical_and(t >= HKV, t < NSTEP))
        def _():
            copy(kind, 1, hk, slot).start()

    def wait(kind, t):
        slot = t % NB if isinstance(t, int) else t & (NB - 1)
        copy(kind, 0, 0, slot).wait()

    def half_slot(t):
        if isinstance(t, int):
            return t // HKV, t % NB
        return t >> 4, t & (NB - 1)

    def x_part(h, lo, hi, sem):
        return pltpu.make_async_copy(halves[h][0].at[pl.ds(lo, hi - lo)], xT_s.at[h, pl.ds(lo, hi - lo)],
                                     sem_x.at[sem])

    def kv_part(kind, lo, hi, sem):
        src = halves[0][1 if kind == "k" else 2]
        dst = k_s if kind == "k" else v_s
        return pltpu.make_async_copy(src.at[pl.ds(lo, hi - lo), 0], dst.at[0, pl.ds(lo, hi - lo)], sem_x.at[sem])

    def xpose_x(h, lo, hi):
        for b in range(lo, hi):
            x_s[h, pl.ds(b * SQ, SQ), :] = xT_s[h, b].T

    def st32(ref, h, r0, val):
        ref[h, pl.ds(r0 // 2, val.shape[0] // 2), :] = pltpu.bitcast(val, U32)

    def ld32(ref, h, r0, n):
        return pltpu.bitcast(ref[h, pl.ds(r0 // 2, n // 2), :], BF)

    def qproj_chunk(t, c, nchunk):
        half, slot = half_slot(t)
        n = R // nchunk
        q = jnp.dot(x_s[half, pl.ds(c * n, n), :], wq_s[slot], preferred_element_type=F32) * SCALE
        q = q.astype(BF)
        st32(q_s, 0, c * n, q[:, :DH])
        st32(q_s, 1, c * n, q[:, DH:])

    def qproj(t):
        qproj_chunk(t, 0, 2)
        qproj_chunk(t, 1, 2)

    def attn_scores(t, b):
        _, slot = half_slot(t)
        q = jnp.concatenate([ld32(q_s, 0, b * SQ, SQ), ld32(q_s, 1, b * SQ, SQ)], axis=0)
        s = jax.lax.dot_general(q, k_s[slot, b], NT, preferred_element_type=F32)
        m = jnp.max(s, axis=1, keepdims=True)
        p = jnp.exp2(s - m)
        l = jnp.sum(p, axis=1, keepdims=True)
        r = pltpu.reciprocal(l, approx=True)
        r = r * (2.0 - l * r)
        return p.astype(BF), r

    def attn_values(t, b, pr):
        _, slot = half_slot(t)
        p, r = pr
        o = jnp.dot(p, v_s[slot, b], preferred_element_type=F32)
        o = (o * r).astype(BF)
        st32(o_s, 0, b * SQ, o[:SQ])
        st32(o_s, 1, b * SQ, o[SQ:])

    def attn(t, lo=0, hi=B):
        pr = {}
        for b in range(lo, hi + 1):
            if b < hi:
                pr[b] = attn_scores(t, b)
            if b > lo:
                attn_values(t, b - 1, pr.pop(b - 1))

    def oproj(t):
        half, slot = half_slot(t)
        o = jnp.concatenate([ld32(o_s, 0, 0, R), ld32(o_s, 1, 0, R)], axis=1)
        acc[1 - half] += jax.lax.dot_general(wo_s[slot], o, NT, preferred_element_type=F32)

    xb0, xb1, xa = x_part(0, 0, 4, 0), x_part(0, 4, 8, 1), x_part(1, 0, 8, 2)
    k0a, v0a = kv_part("k", 0, 4, 3), kv_part("v", 0, 4, 4)
    k0b, v0b = kv_part("k", 4, 8, 5), kv_part("v", 4, 8, 6)
    xb0.start()
    start("wq", 0)
    xb1.start()
    acc[...] = jnp.zeros(acc.shape, F32)
    xb0.wait()
    wait("wq", 0)
    k0a.start()
    v0a.start()
    xpose_x(0, 0, 4)
    for b in range(0, 4):
        qproj_chunk(0, b, B)
    xb1.wait()
    k0b.start()
    v0b.start()
    xpose_x(0, 4, 8)
    for b in range(4, 8):
        qproj_chunk(0, b, B)
    k0a.wait()
    v0a.wait()
    start("wo", 0)
    start("wq", 1)
    attn(0, 0, 4)
    k0b.wait()
    v0b.wait()
    wait("wo", 0)
    start("k", 1)
    start("v", 1)
    attn(0, 4, 8)
    start("wo", 1)
    start("wq", 2)
    oproj(0)
    wait("wq", 1)
    start("k", 2)
    xa.start()
    qproj(1)
    wait("k", 1)
    wait("v", 1)
    wait("wo", 1)
    start("v", 2)
    start("wo", 2)
    attn(1, 0, 4)
    start("wq", 3)
    start("k", 3)
    attn(1, 4, 8)
    oproj(1)
    for kind in KINDS:
        wait(kind, 2)
    xa.wait()
    start("v", 3)
    start("wo", 3)
    xpose_x(1, 0, 8)
    qproj(2)
    for kind in KINDS:
        start(kind, 4)
    attn(2)
    oproj(2)

    def loop_body(i, carry):
        t0 = P + i * U
        for u in range(U):
            for kind in KINDS:
                wait(kind, t0 + u)
        qproj_chunk(t0, 0, 2)
        for u in range(U):
            for kind in KINDS:
                start(kind, t0 + u + U)
        qproj_chunk(t0, 1, 2)
        for u in range(U):
            if u > 0:
                qproj(t0 + u)
            attn(t0 + u)
            oproj(t0 + u)
        return carry

    jax.lax.fori_loop(0, (NSTEP - 1 - P) // U, loop_body, None)

    t = NSTEP - 1
    slot = t % NB
    wait("wq", t)
    for b in range(B):
        rows = pl.ds(b * SQ, SQ)
        out_s[rows, 640:1152] = acc[1, 64:576, rows].astype(BF).T
    copy_b = pltpu.make_async_copy(out_s.at[:, pl.ds(640, 512)], out_hbm.at[:, pl.ds(640, 512)], sem_out.at[0])
    copy_b.start()
    qproj(t)
    wait("k", t)
    wait("v", t)
    wait("wo", t)

    def finish(b):
        rows = pl.ds(b * SQ, SQ)
        o = jnp.concatenate([ld32(o_s, 0, b * SQ, SQ), ld32(o_s, 1, b * SQ, SQ)], axis=1)
        parts = []
        for r in range(2):
            rr = pl.ds(r * (D // 2), D // 2)
            parts.append(acc[0, rr, rows]
                         + jax.lax.dot_general(wo_s[slot, rr, :], o, NT, preferred_element_type=F32))
        out_t = jnp.concatenate(parts + [acc[1, 0:64, rows]], axis=0).astype(BF)
        out_s[rows, 0:640] = out_t.T
        pltpu.make_async_copy(out_s.at[rows, pl.ds(0, 640)], out_hbm.at[rows, pl.ds(0, 640)], sem_out.at[1]).start()

    pr = {}
    for b in range(B + 3):
        if b < B:
            pr[b] = attn_scores(t, b)
        if 1 <= b <= B:
            attn_values(t, b - 1, pr.pop(b - 1))
        if b >= 3:
            finish(b - 3)
    copy_b.wait()
    pltpu.make_async_copy(out_s.at[:, pl.ds(0, 640)], out_hbm.at[:, pl.ds(0, 640)], sem_out.at[1]).wait()


@jax.jit
def pallas_concat_heads__gqa_block_cached__gqa_block_cached__near_ridge_kernel(
    A_x: jax.Array,
    A_k_cache: jax.Array,
    A_v_cache: jax.Array,
    A_wq: jax.Array,
    A_wo: jax.Array,
    B_x: jax.Array,
    B_k_cache: jax.Array,
    B_v_cache: jax.Array,
    B_wq: jax.Array,
    B_wo: jax.Array,
):
    hbm = pl.BlockSpec(memory_space=pltpu.HBM)
    out = pl.pallas_call(
        _kernel,
        out_shape=jax.ShapeDtypeStruct((R, 2 * D), BF),
        in_specs=[hbm] * 10,
        out_specs=hbm,
        scratch_shapes=[
            pltpu.VMEM((2, B, D, SQ), BF),
            pltpu.VMEM((2, R, D), BF),
            pltpu.VMEM((NB, D, 256), BF),
            pltpu.VMEM((NB, D, 256), BF),
            pltpu.VMEM((NB, B, SK, DH), BF),
            pltpu.VMEM((NB, B, SK, DH), BF),
            pltpu.VMEM((2, R // 2, DH), U32),
            pltpu.VMEM((2, R // 2, DH), U32),
            pltpu.VMEM((2, D, R), F32),
            pltpu.VMEM((R, 2 * D), BF),
            pltpu.SemaphoreType.DMA((7,)),
            pltpu.SemaphoreType.DMA((NB,)),
            pltpu.SemaphoreType.DMA((NB,)),
            pltpu.SemaphoreType.DMA((NB,)),
            pltpu.SemaphoreType.DMA((NB,)),
            pltpu.SemaphoreType.DMA((2,)),
        ],
        compiler_params=pltpu.CompilerParams(vmem_limit_bytes=64 * 1024 * 1024, disable_bounds_checks=True),
    )(jnp.transpose(A_x, (0, 2, 1)), A_k_cache, A_v_cache, A_wq, A_wo.T,
      jnp.transpose(B_x, (0, 2, 1)), B_k_cache, B_v_cache, B_wq, B_wo.T)
    return out.reshape(B, SQ, 2 * D)
```
